```python
import os as _os
_os.environ.setdefault("JAX_PLATFORMS", "cpu")
import jax
import jax.numpy as jnp

def _softmax(x, axis=-1):
    return jax.nn.softmax(x, axis=axis)
def _gelu(x):
    return jax.nn.gelu(x, approximate=True)
def _silu(x):
    return jax.nn.silu(x)
def _sigmoid(x):
    return jax.nn.sigmoid(x)
def _layernorm(x, axis=-1, eps=1e-5):
    m = jnp.mean(x, axis=axis, keepdims=True)
    v = jnp.var(x, axis=axis, keepdims=True)
    return (x - m) / jnp.sqrt(v + eps)
def _scatter_add(tgt, idx, src, axis=0):
    return tgt.at[idx].add(src)
def _segment_sum(src, seg, n):
    return jax.ops.segment_sum(src, seg, n)
class _Rng:
    def __init__(self, key):
        self._k = key
    def _next(self):
        self._k, sub = jax.random.split(self._k)
        return sub
    def normal(self, shape):
        return jax.random.normal(self._next(), shape, dtype=jnp.bfloat16)
    def randint(self, lo, hi, shape):
        return jax.random.randint(self._next(), shape, lo, hi, dtype=jnp.int32)
    def uniform(self, shape, lo=0.0, hi=1.0):
        return jax.random.uniform(self._next(), shape, jnp.bfloat16, lo, hi)
    def permutation(self, n):
        return jax.random.permutation(self._next(), n)


kernel_name = 'gated_mix__sliding_block__dense_activation_silu__prompt'

def setup_inputs():
    _rng = _Rng(jax.random.key(int.from_bytes(__import__("os").urandom(4), "little")))
    _w = (lambda a: (lambda t: t.astype(jnp.bfloat16) if jnp.issubdtype(t.dtype, jnp.floating) else t)(jnp.asarray(a)))
    def _A_setup():
        B, S, D = 1, 2048, 640
        return {
            "x": _w((lambda *s: _rng.normal(s) * 0.05)(B, S, D)),
            "wqkv": _w((lambda *s: _rng.normal(s) * 0.4)(D, 3 * D)),
            "wo": _w((lambda *s: _rng.normal(s) * 0.05)(D, D)),
        }
    _A_in = _A_setup()

    def _B_setup():
        B, S, D, F = 1, 2048, 640, 1536
        return {
            "x": _w((lambda *s: _rng.normal(s) * 0.05)(B, S, D)),
            "w1": _w((lambda *s: _rng.normal(s) * 1.6)(D, F) * (D ** -0.5)),
            "w2": _w((lambda *s: _rng.normal(s) * 1.6)(F, D) * (F ** -0.5)),
        }
    _B_in = _B_setup()

    return {
        "A_x": _A_in["x"],
        "A_wqkv": _A_in["wqkv"],
        "A_wo": _A_in["wo"],
        "B_x": _B_in["x"],
        "B_w1": _B_in["w1"],
        "B_w2": _B_in["w2"],
        "gate_w": _w((lambda *s: _rng.normal(s) * 0.05)(640) * 16.0),
    }

def reference(A_x, A_wqkv, A_wo, B_x, B_w1, B_w2, gate_w):
    def _A_ref(x, wqkv, wo):
        B, S, D = x.shape
        H = 32; Dh = D // H; W = 256
        qkv = (lambda x, *d: x.transpose(*d))((x @ wqkv).reshape(B, S, 3, H, Dh), 2, 0, 3, 1, 4)
        q, k, v = qkv[0], qkv[1], qkv[2]
        scores = jnp.einsum("bhqd,bhkd->bhqk", q, k) * (Dh ** -0.5)
        idx = jnp.arange(S)
        mask = (idx[:, None] - idx[None, :] >= 0) & (idx[:, None] - idx[None, :] < W)
        scores = jnp.where(mask[None, None], scores, -1e9)
        p = _softmax(scores, axis=-1)
        o = jnp.einsum("bhqk,bhkd->bhqd", p, v)
        return (lambda x, *d: x.transpose(*d))(o, 0, 2, 1, 3).reshape(B, S, D) @ wo

    def _B_ref(x, w1, w2):
        h = jnp.einsum("bsd,df->bsf", x, w1)
        h = _silu(h)
        out = jnp.einsum("bsf,fd->bsd", h, w2)
        return out

    x = A_x
    g = _sigmoid((x * gate_w).sum(-1, keepdims=True))
    a = _A_ref(x, A_wqkv, A_wo)
    b = _B_ref(x, B_w1, B_w2)
    return g * a + (1 - g) * b
```

```python
import functools
import math

import jax
import jax.numpy as jnp
import jax.experimental.pallas as pl
import jax.experimental.pallas.tpu as pltpu

H = 32
W = 256
QB = 128
KW = W + QB
LOG2E = math.log2(math.e)
NEG = -1e9 * LOG2E


def _kernel(x_ref, wqkv_ref, wo_ref, w1_ref, w2_ref, gw_ref, o_ref,
            k_scr, vt_scr, wvt_scr, ot_scr, *, T, D):
    i = pl.program_id(0)
    dh = D // H
    f32, bf16 = jnp.float32, jnp.bfloat16

    @pl.when(i == 0)
    def _():
        k_scr[0:W, :] = jnp.zeros((W, D), bf16)
        vt_scr[:, 0:W] = jnp.zeros((D, W), bf16)
        wvt_scr[...] = wqkv_ref[:, 2 * D:3 * D].astype(f32).T.astype(bf16)

    xb = x_ref[...]
    row0 = pl.multiple_of(i * T, T)
    qk = jnp.dot(xb, wqkv_ref[:, 0:2 * D], preferred_element_type=f32)
    q = qk[:, 0:D] * (dh ** -0.5 * LOG2E)
    k_scr[pl.ds(W + row0, T), :] = qk[:, D:2 * D].astype(bf16)
    vt = jax.lax.dot_general(wvt_scr[...], xb, (((1,), (1,)), ((), ())),
                             preferred_element_type=f32)
    vt_scr[:, pl.ds(W + row0, T)] = vt.astype(bf16)

    ki = jax.lax.broadcasted_iota(jnp.int32, (QB, QB), 0)
    qj = jax.lax.broadcasted_iota(jnp.int32, (QB, QB), 1)

    a_parts = []
    for j in range(T // QB):
        q0 = row0 + j * QB
        qj_blk = q[j * QB:(j + 1) * QB, :]
        kwin = k_scr[pl.ds(pl.multiple_of(q0, QB), KW), :]
        m0 = jnp.logical_and(ki > qj, q0 >= 2 * QB)
        m1 = (ki >= 0) & (q0 >= QB)
        m2 = ki <= qj
        for h in range(H):
            lo, hi = h * dh, (h + 1) * dh
            c0, c1 = lo // QB, (hi - 1) // QB
            nc = c1 - c0 + 1
            cl, ch = c0 * QB, (c1 + 1) * QB
            lm = jax.lax.broadcasted_iota(jnp.int32, (QB, nc * QB), 1) + cl
            qm = jnp.where((lm >= lo) & (lm < hi), qj_blk[:, cl:ch], 0.0).astype(bf16)
            s = jax.lax.dot_general(kwin[:, cl:ch], qm, (((1,), (1,)), ((), ())),
                                    preferred_element_type=f32)
            s0 = jnp.where(m0, s[0:QB], NEG)
            s1 = jnp.where(m1, s[QB:2 * QB], NEG)
            s2 = jnp.where(m2, s[2 * QB:3 * QB], NEG)
            mx = jnp.max(jnp.maximum(jnp.maximum(s0, s1), s2), axis=0, keepdims=True)
            p = jnp.exp2(jnp.concatenate([s0, s1, s2], axis=0) - mx)
            l = jnp.sum(p, axis=0, keepdims=True)
            r0 = (lo // 16) * 16
            vth = vt_scr[r0:r0 + 32, pl.ds(pl.multiple_of(q0, QB), KW)]
            ot = jnp.dot(vth, p.astype(bf16), preferred_element_type=f32)
            ot = ot * (1.0 / l)
            ot_scr[lo:hi, :] = ot[lo - r0:hi - r0, :]
        o = ot_scr[...].T.astype(bf16)
        a_parts.append(jnp.dot(o, wo_ref[...], preferred_element_type=f32))
    a = jnp.concatenate(a_parts, axis=0)

    hh = jnp.dot(xb, w1_ref[...], preferred_element_type=f32)
    hh = hh * jax.nn.sigmoid(hh)
    b = jnp.dot(hh.astype(bf16), w2_ref[...], preferred_element_type=f32)

    g = jax.nn.sigmoid(jnp.sum(xb.astype(f32) * gw_ref[...].astype(f32), axis=-1, keepdims=True))
    o_ref[...] = (g * a + (1.0 - g) * b).astype(o_ref.dtype)


@jax.jit
def pallas_gated_mix__sliding_block__dense_activation_silu__prompt_kernel(
    A_x: jax.Array,
    A_wqkv: jax.Array,
    A_wo: jax.Array,
    B_x: jax.Array,
    B_w1: jax.Array,
    B_w2: jax.Array,
    gate_w: jax.Array,
):
    B, S, D = A_x.shape
    F = B_w1.shape[1]
    T = 256
    x2 = A_x.reshape(S, D)
    gw = gate_w.reshape(1, D)
    const = lambda i: (0, 0)
    out = pl.pallas_call(
        functools.partial(_kernel, T=T, D=D),
        grid=(S // T,),
        in_specs=[
            pl.BlockSpec((T, D), lambda i: (i, 0)),
            pl.BlockSpec((D, 3 * D), const),
            pl.BlockSpec((D, D), const),
            pl.BlockSpec((D, F), const),
            pl.BlockSpec((F, D), const),
            pl.BlockSpec((1, D), const),
        ],
        out_specs=pl.BlockSpec((T, D), lambda i: (i, 0)),
        out_shape=jax.ShapeDtypeStruct((S, D), A_x.dtype),
        scratch_shapes=[
            pltpu.VMEM((S + W, D), jnp.bfloat16),
            pltpu.VMEM((D, S + W), jnp.bfloat16),
            pltpu.VMEM((D, D), jnp.bfloat16),
            pltpu.VMEM((D, QB), jnp.float32),
        ],
        compiler_params=pltpu.CompilerParams(
            dimension_semantics=("arbitrary",),
            vmem_limit_bytes=64 * 1024 * 1024,
        ),
    )(x2, A_wqkv, A_wo, B_w1, B_w2, gw)
    return out.reshape(B, S, D)
```

```python
import functools
import math

import jax
import jax.numpy as jnp
import jax.experimental.pallas as pl
import jax.experimental.pallas.tpu as pltpu

H = 32
W = 256
QB = 128
T = 256
FC = 128
LOOK = 2
LOG2E = math.log2(math.e)
NEG = -1e9 * LOG2E


def _kernel(x_ref, wqkv_hbm, wo_hbm, w1_hbm, w2_hbm, gw_ref, o_ref,
            wqk_v, wv_v, wo_v, w1_v, w2_v, sems,
            k_scr, vt_scr, wvt_scr, ot_scr, h_scr, tri_scr, b_scr, g_scr, *, D, F, NSTEP):
    i = pl.program_id(0)
    dh = D // H
    f32, bf16, u32 = jnp.float32, jnp.bfloat16, jnp.uint32
    NC = D // QB
    NQ = T // QB

    cp_qk = pltpu.make_async_copy(wqkv_hbm.at[:, 0:2 * D], wqk_v, sems.at[0])
    cp_v = pltpu.make_async_copy(wqkv_hbm.at[:, 2 * D:3 * D], wv_v, sems.at[1])
    cp_w1 = pltpu.make_async_copy(w1_hbm, w1_v, sems.at[2])
    cp_w2 = pltpu.make_async_copy(w2_hbm, w2_v, sems.at[3])
    cp_wo = pltpu.make_async_copy(wo_hbm, wo_v, sems.at[4])

    strad = [h for h in range(H) if (h * dh) // QB != ((h + 1) * dh - 1) // QB]
    groups = {c: [(h, h * dh - c * QB) for h in range(H)
                  if h * dh >= c * QB and (h + 1) * dh <= (c + 1) * QB] for c in range(NC)}
    groups[NC] = [(h, n * dh) for n, h in enumerate(strad)]

    def tail():
        o = ot_scr[...].T.astype(bf16)
        a = jnp.dot(o, wo_v[...], preferred_element_type=f32)
        o_ref[...] = (g_scr[...] * a + b_scr[...]).astype(o_ref.dtype)

    def step(first):
        if first:
            cp_qk.start()
            cp_v.start()
            cp_w1.start()
            cp_w2.start()
            cp_wo.start()
            cp_qk.wait()
        xb = x_ref[...]
        row0 = pl.multiple_of(i * T, T)
        qk = jnp.dot(xb, wqk_v[...], preferred_element_type=f32)
        if not first:
            tail()
        q = qk[:, 0:D] * (dh ** -0.5 * LOG2E)
        kk = qk[:, D:2 * D]
        lane_t = jax.lax.broadcasted_iota(jnp.int32, (T, QB), 1)

        def gather_strad(z):
            out = None
            for n, h in enumerate(strad):
                c = (h * dh) // QB
                pa = h * dh - c * QB
                mrg = jnp.where(lane_t >= pa, z[:, c * QB:(c + 1) * QB], z[:, (c + 1) * QB:(c + 2) * QB])
                mrg = pltpu.roll(mrg, (n * dh - pa) % QB, 1)
                out = mrg if out is None else jnp.where(lane_t >= n * dh, mrg, out)
            return out

        q_x = gather_strad(q)
        k_scr[pl.ds(row0, T), 0:D] = kk.astype(bf16)
        k_scr[pl.ds(row0, T), D:D + QB] = gather_strad(kk).astype(bf16)
        if first:
            cp_v.wait()
            wvt_scr[...] = wv_v[...].astype(f32).T.astype(bf16)
        vt = jax.lax.dot_general(wvt_scr[...], xb, (((1,), (1,)), ((), ())),
                                 preferred_element_type=f32)
        vt_scr[:, pl.ds(row0, T)] = vt.astype(bf16)

        ki = jax.lax.broadcasted_iota(jnp.int32, (QB, QB), 0)
        qj = jax.lax.broadcasted_iota(jnp.int32, (QB, QB), 1)
        lane_h = jax.lax.broadcasted_iota(jnp.int32, (QB // 2, QB), 1)

        g = jax.nn.sigmoid(jnp.sum(xb.astype(f32) * gw_ref[...].astype(f32), axis=-1, keepdims=True))
        g_scr[...] = g

        def ffn1(n):
            if first and n == 0:
                cp_w1.wait()
            hh = jnp.dot(xb, w1_v[:, n * FC:(n + 1) * FC], preferred_element_type=f32)
            h_scr[:, n * FC:(n + 1) * FC] = (hh * jax.nn.sigmoid(hh)).astype(bf16)

        def ffn2(n):
            if first and n == 0:
                cp_w2.wait()
            bb = jnp.dot(h_scr[...], w2_v[:, n * QB:(n + 1) * QB], preferred_element_type=f32)
            b_scr[:, n * QB:(n + 1) * QB] = (1.0 - g) * bb

        fillers = ([functools.partial(ffn1, n) for n in range(F // FC)]
                   + [functools.partial(ffn2, n) for n in range(NC)])
        stages = [(j, cc) for j in range(NQ) for cc in [NC] + list(range(NC))]
        nstage = len(stages)
        sched = [[] for _ in range(nstage + 1)]
        for t, fl in enumerate(fillers):
            sched[min(nstage, int(1.0 + (nstage - 1.0) * t / (len(fillers) - 1)))].append(fl)

        if first:
            tb = pltpu.bitcast(jnp.where(ki > qj, 1.0, 0.0).astype(bf16), u32)
            tm = (jnp.where((tb & u32(0xFFFF)) != 0, u32(0xFFFF), u32(0))
                  | jnp.where((tb >> 16) != 0, u32(0xFFFF0000), u32(0)))
            tri_scr[0] = tm
            tri_scr[1] = ~tm

        def window(j):
            nt = min(3, j + 1) if first else 3
            return nt, pl.multiple_of(row0 + (j + 1 - nt) * QB, QB)

        kwins = {}

        def qk_stage(j, cc):
            nt, k0 = window(j)
            if j not in kwins:
                kwin = k_scr[pl.ds(k0, nt * QB), :]
                if nt == 3:
                    kwin = jnp.concatenate(
                        [kwin[o + 16 * r:o + 16 * r + 16] for r in range(QB // 16) for o in (0, 2 * QB)]
                        + [kwin[QB:2 * QB]], axis=0)
                kwins[j] = kwin
            qsrc = q_x[j * QB:(j + 1) * QB, :] if cc == NC else q[j * QB:(j + 1) * QB, cc * QB:(cc + 1) * QB]
            qc = pltpu.bitcast(qsrc.astype(bf16), u32)
            qm = jnp.concatenate(
                [pltpu.bitcast(jnp.where((lane_h >= off) & (lane_h < off + dh), qc, u32(0)), bf16)
                 for _, off in groups[cc]], axis=0)
            return jax.lax.dot_general(kwins[j][:, cc * QB:(cc + 1) * QB], qm, (((1,), (1,)), ((), ())),
                                       preferred_element_type=f32)

        def sm_stage(j, cc, sc):
            nt, k0 = window(j)
            for n, (h, _) in enumerate(groups[cc]):
                lo, hi = h * dh, (h + 1) * dh
                s = sc[:, n * QB:(n + 1) * QB]
                if nt == 3:
                    s_old = jnp.concatenate([s[32 * r:32 * r + 16] for r in range(QB // 16)], axis=0)
                    s_dia = jnp.concatenate([s[32 * r + 16:32 * r + 32] for r in range(QB // 16)], axis=0)
                    s_mid = s[2 * QB:3 * QB]
                    sm = jnp.where(ki > qj, s_old, s_dia)
                    mx = jnp.max(jnp.maximum(sm, s_mid), axis=0, keepdims=True)
                    pm = pltpu.bitcast(jnp.exp2(sm - mx).astype(bf16), u32)
                    p1 = jnp.exp2(s_mid - mx).astype(bf16)
                    pb = jnp.concatenate([pltpu.bitcast(pm & tri_scr[0], bf16), p1,
                                          pltpu.bitcast(pm & tri_scr[1], bf16)], axis=0)
                else:
                    tiles = [s[t * QB:(t + 1) * QB] for t in range(nt)]
                    tiles[-1] = jnp.where(ki <= qj, tiles[-1], NEG)
                    mx = jnp.max(functools.reduce(jnp.maximum, tiles), axis=0, keepdims=True)
                    pb = jnp.exp2(jnp.concatenate(tiles, axis=0) - mx).astype(bf16)
                r0 = (lo // 16) * 16
                rr = {0: 10, 4: 12, 8: 14, 12: 0}[lo - r0]
                vu = pltpu.bitcast(vt_scr[r0:r0 + 32, pl.ds(k0, nt * QB)], u32)
                vu = jnp.where(jax.lax.broadcasted_iota(jnp.int32, vu.shape, 0) == rr,
                               u32(0x3F803F80), vu)
                ot = jnp.dot(pltpu.bitcast(vu, bf16), pb, preferred_element_type=f32)
                ot = ot * (1.0 / ot[2 * rr:2 * rr + 1, :])
                ot_scr[lo:hi, j * QB:(j + 1) * QB] = ot[lo - r0:hi - r0, :]

        scs = {}
        for t in range(min(LOOK, nstage)):
            scs[t] = qk_stage(*stages[t])
        for t, (j, cc) in enumerate(stages):
            if t + LOOK < nstage:
                scs[t + LOOK] = qk_stage(*stages[t + LOOK])
            for fl in sched[t]:
                fl()
            sm_stage(j, cc, scs.pop(t))
        for fl in sched[nstage]:
            fl()
        if first:
            cp_wo.wait()

    @pl.when(i == 0)
    def _():
        step(True)

    @pl.when(jnp.logical_and(i > 0, i < NSTEP))
    def _():
        step(False)

    @pl.when(i == NSTEP)
    def _():
        tail()


@jax.jit
def pallas_gated_mix__sliding_block__dense_activation_silu__prompt_kernel(
    A_x: jax.Array,
    A_wqkv: jax.Array,
    A_wo: jax.Array,
    B_x: jax.Array,
    B_w1: jax.Array,
    B_w2: jax.Array,
    gate_w: jax.Array,
):
    B, S, D = A_x.shape
    F = B_w1.shape[1]
    assert B == 1 and S % T == 0 and W == 2 * QB and T >= W and D % QB == 0 and F % FC == 0
    nstep = S // T
    x2 = A_x.reshape(S, D)
    gw = gate_w.reshape(1, D)
    anyspec = pl.BlockSpec(memory_space=pl.ANY)
    bf16 = jnp.bfloat16
    out = pl.pallas_call(
        functools.partial(_kernel, D=D, F=F, NSTEP=nstep),
        grid=(nstep + 1,),
        in_specs=[
            pl.BlockSpec((T, D), lambda i: (jnp.minimum(i, nstep - 1), 0)),
            anyspec, anyspec, anyspec, anyspec,
            pl.BlockSpec((1, D), lambda i: (0, 0)),
        ],
        out_specs=pl.BlockSpec((T, D), lambda i: (jnp.maximum(i - 1, 0), 0)),
        out_shape=jax.ShapeDtypeStruct((S, D), A_x.dtype),
        scratch_shapes=[
            pltpu.VMEM((D, 2 * D), bf16),
            pltpu.VMEM((D, D), bf16),
            pltpu.VMEM((D, D), bf16),
            pltpu.VMEM((D, F), bf16),
            pltpu.VMEM((F, D), bf16),
            pltpu.SemaphoreType.DMA((5,)),
            pltpu.VMEM((S, D + QB), bf16),
            pltpu.VMEM((D, S), bf16),
            pltpu.VMEM((D, D), bf16),
            pltpu.VMEM((D, T), jnp.float32),
            pltpu.VMEM((T, F), bf16),
            pltpu.VMEM((2, QB // 2, QB), jnp.uint32),
            pltpu.VMEM((T, D), jnp.float32),
            pltpu.VMEM((T, 1), jnp.float32),
        ],
        compiler_params=pltpu.CompilerParams(
            dimension_semantics=("arbitrary",),
            vmem_limit_bytes=64 * 1024 * 1024,
        ),
    )(x2, A_wqkv, A_wo, B_w1, B_w2, gw)
    return out.reshape(B, S, D)
```

```python
import functools
import math

import jax
import jax.numpy as jnp
import jax.experimental.pallas as pl
import jax.experimental.pallas.tpu as pltpu

H = 32
W = 256
QB = 128
T = 256
FC = 128
LOOK = 12
LOG2E = math.log2(math.e)
NEG = -1e9 * LOG2E


def _kernel(x_ref, wqkv_hbm, wo_hbm, w1_hbm, w2_hbm, gw_ref, o_ref,
            wqk_v, wv_v, wo_v, w1_v, w2_v, sems,
            k_scr, vt_scr, wvt_scr, ot_scr, h_scr, tri_scr, b_scr, g_scr, q_scr, pm_scr, *, D, F, NSTEP):
    i = pl.program_id(0)
    dh = D // H
    f32, bf16, u32 = jnp.float32, jnp.bfloat16, jnp.uint32
    NC = D // QB
    NQ = T // QB

    cp_q = pltpu.make_async_copy(wqkv_hbm.at[:, 0:D], wqk_v.at[:, 0:D], sems.at[0])
    cp_k = pltpu.make_async_copy(wqkv_hbm.at[:, D:2 * D], wqk_v.at[:, D:2 * D], sems.at[5])
    cp_v = pltpu.make_async_copy(wqkv_hbm.at[:, 2 * D:3 * D], wv_v, sems.at[1])
    cp_w1 = pltpu.make_async_copy(w1_hbm, w1_v, sems.at[2])
    cp_w2 = pltpu.make_async_copy(w2_hbm, w2_v, sems.at[3])
    cp_wo = pltpu.make_async_copy(wo_hbm, wo_v, sems.at[4])

    HG = (QB // 2) // dh
    NG = -(-H // HG)
    groups = {m: [(h, (h - m * HG) * dh) for h in range(m * HG, min(H, (m + 1) * HG))] for m in range(NG)}

    def tail():
        o = ot_scr[...].T.astype(bf16)
        a = jnp.dot(o, wo_v[...], preferred_element_type=f32)
        o_ref[...] = (g_scr[...] * a + b_scr[...]).astype(o_ref.dtype)

    def step(first):
        if first:
            cp_k.start()
            cp_v.start()
            cp_q.start()
            cp_w1.start()
            cp_w2.start()
            cp_wo.start()
            cp_k.wait()
        xb = x_ref[...]
        row0 = pl.multiple_of(i * T, T)
        if first:
            kk = jnp.dot(xb, wqk_v[:, D:2 * D], preferred_element_type=f32)
            cp_v.wait()
            cp_q.wait()
            wvt_scr[...] = wv_v[...].astype(f32).T.astype(bf16)
            q = jnp.dot(xb, wqk_v[:, 0:D], preferred_element_type=f32)
        else:
            qk = jnp.dot(xb, wqk_v[...], preferred_element_type=f32)
            tail()
            q, kk = qk[:, 0:D], qk[:, D:2 * D]
        q = q * (dh ** -0.5 * LOG2E)
        lane_t = jax.lax.broadcasted_iota(jnp.int32, (T, QB), 1)

        def half_chunks(z, m):
            lo = m * HG * dh
            c, o = lo // QB, lo % QB
            n = len(groups[m]) * dh
            mrg = z[:, c * QB:(c + 1) * QB]
            if o + n > QB:
                mrg = jnp.where(lane_t >= o, mrg, z[:, (c + 1) * QB:(c + 2) * QB])
            low = mrg if o == 0 else pltpu.roll(mrg, (-o) % QB, 1)
            high = mrg if o == QB // 2 else pltpu.roll(mrg, (QB // 2 - o) % QB, 1)
            return jnp.where(lane_t < QB // 2, low, high)

        for m in range(NG):
            q_scr[:, m * QB:(m + 1) * QB] = half_chunks(q, m).astype(bf16)
            k_scr[pl.ds(row0, T), m * QB:(m + 1) * QB] = half_chunks(kk, m).astype(bf16)
        vt = jax.lax.dot_general(wvt_scr[...], xb, (((1,), (1,)), ((), ())),
                                 preferred_element_type=f32)
        vt_scr[:, pl.ds(row0, T)] = vt.astype(bf16)

        ki = jax.lax.broadcasted_iota(jnp.int32, (QB, QB), 0)
        qj = jax.lax.broadcasted_iota(jnp.int32, (QB, QB), 1)
        lane_h = jax.lax.broadcasted_iota(jnp.int32, (QB // 2, QB), 1)

        g = jax.nn.sigmoid(jnp.sum(xb.astype(f32) * gw_ref[...].astype(f32).reshape(1, D), axis=-1, keepdims=True))
        g_scr[...] = g

        def ffn1(n):
            if first and n == 0:
                cp_w1.wait()
            hh = jnp.dot(xb, w1_v[:, n * FC:(n + 1) * FC], preferred_element_type=f32)
            hu = 0.5 * hh
            h_scr[:, n * FC:(n + 1) * FC] = (hu * jnp.tanh(hu) + hu).astype(bf16)

        def ffn2(n):
            if first and n == 0:
                cp_w2.wait()
            bb = jnp.dot(h_scr[...], w2_v[:, n * QB:(n + 1) * QB], preferred_element_type=f32)
            b_scr[:, n * QB:(n + 1) * QB] = (1.0 - g) * bb

        fillers = ([functools.partial(ffn1, n) for n in range(F // FC)]
                   + [functools.partial(ffn2, n) for n in range(NC)])
        stages = [(j, cc) for j in range(NQ) for cc in range(NG)]
        nstage = len(stages)
        sched = [[] for _ in range(nstage + 1)]
        for t, fl in enumerate(fillers):
            sched[2 + (nstage - 2) * t // (len(fillers) - 1)].append(fl)

        if first:
            tb = pltpu.bitcast(jnp.where(ki > qj, 1.0, 0.0).astype(bf16), u32)
            tm = (jnp.where((tb & u32(0xFFFF)) != 0, u32(0xFFFF), u32(0))
                  | jnp.where((tb >> 16) != 0, u32(0xFFFF0000), u32(0)))
            tri_scr[0] = tm
            tri_scr[1] = ~tm

        def window(j):
            nt = min(3, j + 1) if first else 3
            return nt, pl.multiple_of(row0 + (j + 1 - nt) * QB, QB)

        HQ = QB // 2
        row_h = jax.lax.broadcasted_iota(jnp.int32, (QB // 2, QB), 0)
        lane_sh = lane_h - jnp.where(row_h >= QB // 4, HQ, 0)
        lane_q = jax.lax.broadcasted_iota(jnp.int32, (HQ // 2, QB), 1)

        def qk_stage(j, cc):
            nt, k0 = window(j)
            cols = slice(cc * QB, (cc + 1) * QB)
            qc = pltpu.bitcast(q_scr[j * QB:(j + 1) * QB, cols], u32)
            def masked(lanes):
                return jnp.concatenate(
                    [pltpu.bitcast(jnp.where((lanes >= off) & (lanes < off + dh), qc, u32(0)), bf16)
                     for _, off in groups[cc]], axis=0)
            dn = (((1,), (1,)), ((), ()))
            if nt < 3:
                return (jax.lax.dot_general(k_scr[pl.ds(k0, nt * QB), cols], masked(lane_h), dn,
                                            preferred_element_type=f32), None)
            ka = pltpu.bitcast(k_scr[pl.ds(k0, HQ), cols], u32)
            kb = pltpu.bitcast(k_scr[pl.ds(pl.multiple_of(k0 + 5 * HQ, HQ), HQ), cols], u32)
            kc = pltpu.bitcast(jnp.where(lane_q < HQ, ka, kb), bf16)
            s_c = jax.lax.dot_general(kc, masked(lane_sh), dn, preferred_element_type=f32)
            s_a = jax.lax.dot_general(k_scr[pl.ds(pl.multiple_of(k0 + HQ, HQ), 4 * HQ), cols], masked(lane_h), dn,
                                      preferred_element_type=f32)
            return s_a, s_c

        def sm_stage(j, cc, sc):
            nt, k0 = window(j)
            for n, (h, _) in enumerate(groups[cc]):
                lo, hi = h * dh, (h + 1) * dh
                s = sc[0][:, n * QB:(n + 1) * QB]
                if nt == 3:
                    s_c = sc[1][:, n * QB:(n + 1) * QB]
                    s_old = jnp.concatenate([s_c, s[0:HQ]], axis=0)
                    s_dia = jnp.concatenate([s[3 * HQ:4 * HQ], s_c], axis=0)
                    s_mid = s[HQ:3 * HQ]
                    sm = jnp.where(ki > qj, s_old, s_dia)
                    mx = jnp.max(jnp.maximum(sm, s_mid), axis=0, keepdims=True)
                    pm_scr[j * H + h] = jnp.exp2(sm - mx).astype(bf16)
                    pm = pltpu.bitcast(pm_scr[j * H + h], u32)
                    p1 = jnp.exp2(s_mid - mx).astype(bf16)
                    pb = jnp.concatenate([pltpu.bitcast(pm & tri_scr[0], bf16), p1,
                                          pltpu.bitcast(pm & tri_scr[1], bf16)], axis=0)
                else:
                    tiles = [s[t * QB:(t + 1) * QB] for t in range(nt)]
                    tiles[-1] = jnp.where(ki <= qj, tiles[-1], NEG)
                    mx = jnp.max(functools.reduce(jnp.maximum, tiles), axis=0, keepdims=True)
                    pb = jnp.exp2(jnp.concatenate(tiles, axis=0) - mx).astype(bf16)
                r0 = (lo // 16) * 16
                rr = {0: 10, 4: 12, 8: 14, 12: 0}[lo - r0]
                vu = pltpu.bitcast(vt_scr[r0:r0 + 32, pl.ds(k0, nt * QB)], u32)
                vu = jnp.where(jax.lax.broadcasted_iota(jnp.int32, vu.shape, 0) == rr,
                               u32(0x3F803F80), vu)
                ot = jnp.dot(pltpu.bitcast(vu, bf16), pb, preferred_element_type=f32)
                ot = ot * (1.0 / ot[2 * rr:2 * rr + 1, :])
                ot_scr[lo:hi, j * QB:(j + 1) * QB] = ot[lo - r0:hi - r0, :]

        scs = {}
        for t in range(min(LOOK, nstage)):
            scs[t] = qk_stage(*stages[t])
        for t, (j, cc) in enumerate(stages):
            if t + LOOK < nstage:
                scs[t + LOOK] = qk_stage(*stages[t + LOOK])
            for fl in sched[t]:
                fl()
            sm_stage(j, cc, scs.pop(t))
        for fl in sched[nstage]:
            fl()
        if first:
            cp_wo.wait()

    @pl.when(i == 0)
    def _():
        step(True)

    @pl.when(jnp.logical_and(i > 0, i < NSTEP))
    def _():
        step(False)

    @pl.when(i == NSTEP)
    def _():
        tail()


@jax.jit
def pallas_gated_mix__sliding_block__dense_activation_silu__prompt_kernel(
    A_x: jax.Array,
    A_wqkv: jax.Array,
    A_wo: jax.Array,
    B_x: jax.Array,
    B_w1: jax.Array,
    B_w2: jax.Array,
    gate_w: jax.Array,
):
    B, S, D = A_x.shape
    F = B_w1.shape[1]
    assert B == 1 and S % T == 0 and W == 2 * QB and T >= W and D % QB == 0 and F % FC == 0
    assert D == 20 * H
    nstep = S // T
    x2 = A_x.reshape(S, D)
    anyspec = pl.BlockSpec(memory_space=pl.ANY)
    bf16 = jnp.bfloat16
    out = pl.pallas_call(
        functools.partial(_kernel, D=D, F=F, NSTEP=nstep),
        grid=(nstep + 1,),
        in_specs=[
            pl.BlockSpec((T, D), lambda i: (jnp.minimum(i, nstep - 1), 0)),
            anyspec, anyspec, anyspec, anyspec,
            pl.BlockSpec((D,), lambda i: (0,)),
        ],
        out_specs=pl.BlockSpec((T, D), lambda i: (jnp.maximum(i - 1, 0), 0)),
        out_shape=jax.ShapeDtypeStruct((S, D), A_x.dtype),
        scratch_shapes=[
            pltpu.VMEM((D, 2 * D), bf16),
            pltpu.VMEM((D, D), bf16),
            pltpu.VMEM((D, D), bf16),
            pltpu.VMEM((D, F), bf16),
            pltpu.VMEM((F, D), bf16),
            pltpu.SemaphoreType.DMA((6,)),
            pltpu.VMEM((S, -(-H // ((QB // 2) // (D // H))) * QB), bf16),
            pltpu.VMEM((D, S), bf16),
            pltpu.VMEM((D, D), bf16),
            pltpu.VMEM((D, T), jnp.float32),
            pltpu.VMEM((T, F), bf16),
            pltpu.VMEM((2, QB // 2, QB), jnp.uint32),
            pltpu.VMEM((T, D), jnp.float32),
            pltpu.VMEM((T, 1), jnp.float32),
            pltpu.VMEM((T, -(-H // ((QB // 2) // (D // H))) * QB), bf16),
            pltpu.VMEM((T // QB * H, QB, QB), bf16),
        ],
        compiler_params=pltpu.CompilerParams(
            dimension_semantics=("arbitrary",),
            vmem_limit_bytes=64 * 1024 * 1024,
        ),
    )(x2, A_wqkv, A_wo, B_w1, B_w2, gate_w)
    return out.reshape(B, S, D)
```
